```python
import jax
import jax.numpy as jnp

def _softmax(x, axis=-1):
    return jax.nn.softmax(x, axis=axis)
def _gelu(x):
    return jax.nn.gelu(x, approximate=True)
def _silu(x):
    return jax.nn.silu(x)
def _sigmoid(x):
    return jax.nn.sigmoid(x)
def _layernorm(x, axis=-1, eps=1e-5):
    m = jnp.mean(x, axis=axis, keepdims=True)
    v = jnp.var(x, axis=axis, keepdims=True)
    return (x - m) / jnp.sqrt(v + eps)
def _scatter_add(tgt, idx, src, axis=0):
    return tgt.at[idx].add(src)
def _segment_sum(src, seg, n):
    return jax.ops.segment_sum(src, seg, n)
class _Rng:
    def __init__(self, key):
        self._k = key
    def _next(self):
        self._k, sub = jax.random.split(self._k)
        return sub
    def normal(self, shape):
        return jax.random.normal(self._next(), shape, dtype=jnp.bfloat16)
    def randint(self, lo, hi, shape):
        return jax.random.randint(self._next(), shape, lo, hi, dtype=jnp.int32)
    def uniform(self, shape, lo=0.0, hi=1.0):
        return jax.random.uniform(self._next(), shape, jnp.bfloat16, lo, hi)
    def permutation(self, n):
        return jax.random.permutation(self._next(), n)


kernel_name = 'recurrent_scan__linear_kernel_hedgehog__dense_activation_relu__prompt'

def _fwd_setup_inputs():
    _rng = _Rng(jax.random.key(int.from_bytes(__import__("os").urandom(4), "little")))
    _w = (lambda a: (lambda t: t.astype(jnp.bfloat16) if jnp.issubdtype(t.dtype, jnp.floating) else t)(jnp.asarray(a)))
    def _A_setup():
        B, S, D, H = 1, 2048, 1024, 32
        Dh = D // H
        return {
            "x": _w((lambda *s: _rng.normal(s) * 0.05)(B, S, D)),
            "wqkv": _w((lambda *s: _rng.normal(s) * 0.05)(D, 3 * D)),
            "w_phi": _w((lambda *s: _rng.normal(s) * 0.05)(H, Dh, Dh) * (Dh ** -0.5)),
            "wo": _w((lambda *s: _rng.normal(s) * 0.05)(D, D)),
        }
    _A_in = _A_setup()

    def _B_setup():
        B, S, D, Dff = 1, 2048, 1024, 3584
        return {
            "x": _w((lambda *s: _rng.normal(s) * 0.05)(B, S, D)),
            "w1": _w((lambda *s: _rng.normal(s) * 0.05)(D, Dff)),
            "w2": _w((lambda *s: _rng.normal(s) * 0.05)(Dff, D)),
        }
    _B_in = _B_setup()

    return {
        "A_x": _A_in["x"],
        "A_wqkv": _A_in["wqkv"],
        "A_w_phi": _A_in["w_phi"],
        "A_wo": _A_in["wo"],
        "B_x": _B_in["x"],
        "B_w1": _B_in["w1"],
        "B_w2": _B_in["w2"],
    }

def _fwd_reference(A_x, A_wqkv, A_w_phi, A_wo, B_x, B_w1, B_w2):
    def _A_ref(x, wqkv, w_phi, wo):
        B, S, D = x.shape
        H = 32; Dh = D // H
        qkv = (lambda x, *d: x.transpose(*d))((x @ wqkv).reshape(B, S, 3, H, Dh), 2, 0, 3, 1, 4)
        q, k, v = qkv[0], qkv[1], qkv[2]
        pq = jnp.einsum("bhsd,hdf->bhsf", q, w_phi)
        pk = jnp.einsum("bhsd,hdf->bhsf", k, w_phi)
        phi_q = jnp.concatenate([_softmax(pq, axis=-1), _softmax(-pq, axis=-1)], axis=-1)
        phi_k = jnp.concatenate([_softmax(pk, axis=-1), _softmax(-pk, axis=-1)], axis=-1)
        kv = jnp.einsum("bhsf,bhsd->bhfd", phi_k, v)
        z  = jnp.einsum("bhsf->bhf", phi_k)
        num = jnp.einsum("bhqf,bhfd->bhqd", phi_q, kv)
        den = jnp.einsum("bhqf,bhf->bhq", phi_q, z)[..., None] + 1e-6
        o = num / den
        return (lambda x, *d: x.transpose(*d))(o, 0, 2, 1, 3).reshape(B, S, D) @ wo

    def _B_ref(x, w1, w2):
        h = jnp.einsum("bsd,df->bsf", x, w1)
        zero = jnp.zeros_like(h)
        h = jnp.maximum(h, zero)
        return jnp.einsum("bsf,fd->bsd", h, w2)

    x = A_x
    xn = _layernorm(x, axis=-1)
    s = _A_ref(xn, A_wqkv, A_w_phi, A_wo)
    g = _silu(_B_ref(xn, B_w1, B_w2))
    return x + s * g


def setup_inputs():
    _inp = _fwd_setup_inputs()
    _gk = jax.random.fold_in(jax.random.key(int.from_bytes(__import__("os").urandom(4), "little")), 2**31 - 1)
    _shapes = [[1, 2048, 1024]]
    _dtypes = ['bfloat16']
    _gks = jax.random.split(_gk, len(_shapes))
    _gs = [jax.random.normal(k, s, dtype=jnp.dtype(d)) * 0.05 for k, s, d in zip(_gks, _shapes, _dtypes)]
    _inp["grad_out"] = _gs[0]
    return _inp

def reference(A_x, A_wqkv, A_w_phi, A_wo, B_w1, B_w2, B_x, grad_out):
    _const = dict(B_x=B_x)
    def _f(*_d):
        return _fwd_reference(**{'A_x': _d[0], 'A_wqkv': _d[1], 'A_w_phi': _d[2], 'A_wo': _d[3], 'B_w1': _d[4], 'B_w2': _d[5], **_const})
    _out, _vjp = jax.vjp(_f, A_x, A_wqkv, A_w_phi, A_wo, B_w1, B_w2)
    _grads = _vjp(grad_out)
    _out0 = jnp.asarray(_out)
    return (_out0, *[jnp.asarray(_g) for _g in _grads])
```

```python
import jax
import jax.numpy as jnp
from jax import lax
import jax.experimental.pallas as pl
import jax.experimental.pallas.tpu as pltpu

S, D, H, DH, DFF = 2048, 1024, 32, 32, 3584
T = 256
NT = S // T
FC = 512
NF = DFF // FC
MF = 1024
NM = S // MF
CB = 512
G = D // 128
NP = H // 2
PLAN_F = "ppdpdpdpd" + "hhhphhhph" + "hhhdhhhdhhhd"
PLAN_B = "hhhhdhhhdhhhdhhhdhhhddd"
BF, F32 = jnp.bfloat16, jnp.float32


def _nn(a, b):
    return lax.dot_general(a, b, (((1,), (0,)), ((), ())), preferred_element_type=F32)


def _nt(a, b):
    return lax.dot_general(a, b, (((1,), (1,)), ((), ())), preferred_element_type=F32)


def _quad(ref, r0, c0, m, n):
    return lambda i, j: ref[pl.ds(r0 + i * m, m), pl.ds(c0 + j * n, n)]


def _lhs7(a):
    terms = (lambda: a(0, 0), lambda: a(0, 0) + a(0, 1), lambda: a(0, 0) + a(1, 1), lambda: a(1, 0) + a(1, 1),
             lambda: a(1, 1), lambda: a(0, 1) - a(1, 1), lambda: a(1, 0) - a(0, 0))
    return lambda n: terms[n]().astype(BF)


def _rhs7(b):
    terms = (lambda: b(0, 1) - b(1, 1), lambda: b(1, 1), lambda: b(0, 0) + b(1, 1), lambda: b(0, 0),
             lambda: b(1, 0) - b(0, 0), lambda: b(1, 0) + b(1, 1), lambda: b(0, 0) + b(0, 1))
    return lambda n: terms[n]().astype(BF)


def _strassen_steps(l, r, dot, c, plain_lhs_first=False):
    m = lambda n: dot(l(n), r(n))
    first = m(0 if plain_lhs_first else 1)
    yield
    m3, m5 = (first, m(1)) if plain_lhs_first else (m(0), first)
    c[0][1] = m3 + m5
    yield
    m1 = m(2)
    c00, c11 = m1 - m5, m1 + m3
    yield
    m4 = m(4)
    c00 = c00 + m4
    yield
    c[0][0] = c00 + m(5)
    yield
    m2 = m(3)
    c[1][0], c11 = m2 + m4, c11 - m2
    yield
    c[1][1] = c11 + m(6)
    yield


def _strassen(l, r, dot, plain_lhs_first=False):
    c = [[None, None], [None, None]]
    for _ in _strassen_steps(l, r, dot, c, plain_lhs_first):
        pass
    return c


def _interleave(plan, **gens):
    for name in plan:
        next(gens[name])


def _blocks(v):
    m, n = v.shape[0] // 2, v.shape[1] // 2
    return lambda i, j: v[i * m:(i + 1) * m, j * n:(j + 1) * n]


def _join(c):
    return jnp.concatenate([jnp.concatenate(row, axis=1) for row in c], axis=0)


def _tr(b):
    return lambda k, j: b(j, k)


_R2L = (5, 4, 2, 0, 6, 3, 1)
_IJ = ((0, 1), (0, 0), (1, 0), (1, 1))


def _iota(shape, d):
    return lax.broadcasted_iota(jnp.int32, shape, d)


def _hred(x, op):
    parts = [x[8 * i:8 * i + 8] for i in range(8)]
    while len(parts) > 1:
        parts = [op(parts[i], parts[i + 1]) for i in range(0, len(parts), 2)]
    r = parts[0]
    r = op(r, pltpu.roll(r, 4, 0))
    return op(r, pltpu.roll(r, 2, 0))


def _tile8(r):
    return jnp.concatenate([r] * 8, axis=0)


def _dual_softmax(p):
    ep = jnp.exp(p - _tile8(_hred(p, jnp.maximum)))
    en = jnp.exp(_tile8(_hred(p, jnp.minimum)) - p)
    return jnp.concatenate([ep * _tile8(1.0 / _hred(ep, jnp.add)),
                            en * _tile8(1.0 / _hred(en, jnp.add))], axis=0).astype(BF)


def _dual_softmax_bwd(phb, dph):
    ph = phb.astype(F32)
    t = ph * dph
    pp, pn, tp, tn = ph[:64], ph[64:], t[:64], t[64:]
    return ((tp - pp * _tile8(_hred(tp, jnp.add))) - (tn - pn * _tile8(_hred(tn, jnp.add)))).astype(BF)


def _head_rows(r):
    return jnp.concatenate([jnp.broadcast_to(r[h:h + 1], (32, r.shape[1])) for h in range(2)], axis=0)


def _head_sums(x):
    s0, s1 = [jnp.broadcast_to(jnp.sum(x[32 * h:32 * h + 32], axis=0, keepdims=True), (16, x.shape[1]))
              for h in range(2)]
    return jnp.where(_iota(s0.shape, 0) % 2 == 0, s0, s1)


def _kernel(x_h, wqkv_h, wphi_ref, wo_h, w1_h, w2_h, go_h,
            out_h, dx_h, dwqkv_h, dwphi_ref, dwo_h, dw1_h, dw2_h,
            xv, gov, wqk, wv, wf7, wo, w1, w2, xn, xn9, rstd, bd, hbuf, phik, dpT,
            du7, kv_acc, dkv_acc, kvb, kvTb, isem, osem):
    off = lambda i, n: i * n if isinstance(i, int) else pl.multiple_of(i * n, n)
    blk = lambda i, n: pl.ds(off(i, n), n)
    HD, HF, HM = D // 2, FC // 2, MF // 2
    relu = lambda v: jnp.maximum(v, 0)
    HT = T // 2

    def put_lhs7(dst, t, vT):
        l = _lhs7(_blocks(vT))
        for n in range(7):
            dst[n, :, blk(t, HT)] = l(n)

    def tok_rows(ref, c0, n, fn=lambda v: v):
        return _rhs7(lambda k, j: fn(jnp.concatenate(
            [ref[pl.ds(t * T + k * HT, HT), pl.ds(c0 + j * n, n)] for t in range(NT)], axis=0)))

    def tok_cols(ref, r0, n):
        return _rhs7(lambda k, j: jnp.concatenate(
            [ref[pl.ds(r0 + j * n, n), pl.ds(t * T + k * HT, HT)] for t in range(NT)], axis=1))

    rows = lambda t: blk(t, T)
    Q, K, VV = pl.ds(0, D), pl.ds(D, D), pl.ds(2 * D, D)
    copy = pltpu.make_async_copy

    x_cp = lambda t: copy(x_h.at[rows(t)], xv.at[rows(t)], isem.at[t])
    wq_cp = copy(wqkv_h.at[:, Q], wqk.at[:, Q], isem.at[NT])
    wk_cp = copy(wqkv_h.at[:, K], wqk.at[:, K], isem.at[NT + 1])
    wv_cp = copy(wqkv_h.at[:, VV], wv, isem.at[NT + 2])
    late_cp = [copy(w1_h, w1, isem.at[NT + 3]), copy(w2_h, w2, isem.at[NT + 4]),
               copy(wo_h, wo, isem.at[NT + 5]), copy(go_h, gov, isem.at[NT + 6])]
    for c in [x_cp(0), wv_cp] + [x_cp(t) for t in range(1, NT)] + [wk_cp, wq_cp] + late_cp:
        c.start()

    col = _iota((128, 128), 1)
    hmask = (_iota((128, 128), 0) // 32) == (col // 64) * 2 + col % 2
    expand = (_iota((32, 128), 0) == (_iota((32, 128), 1) % 64) // 2).astype(BF)
    for g in range(G):
        m = jnp.where(hmask, _nn(wphi_ref[pl.ds(128 * g, 128), :], expand), 0.0)
        bd[g] = m.astype(BF)
        bd[G + g] = m.T.astype(BF)

    def layernorm(t):
        r = rows(t)
        xf = xv[r, :].astype(F32)
        xc = xf - jnp.mean(xf, axis=1, keepdims=True)
        rs = lax.rsqrt(jnp.mean(xc * xc, axis=1, keepdims=True) + 1e-5)
        y = xc * rs
        rstd[r, :] = jnp.broadcast_to(rs, (T, 128))
        xn[r, :] = y.astype(BF)
        yT = y.T
        put_lhs7(xn9, t, yT)
        xn9[7, :, blk(t, HT)] = yT[:HD, HT:].astype(BF)
        xn9[8, :, blk(t, HT)] = yT[HD:, :HT].astype(BF)

    def fold(dst, cs, g):
        w = _nn(wqk[:, cs], bd[g])
        wT = w.T
        l = _lhs7(_blocks(wT))
        for n in range(7):
            dst[n, blk(g, 64), :] = l(n)
        return w

    def project(w7, t):
        cb = [[None, None], [None, None]]
        steps = _strassen_steps(lambda n: w7[n], lambda n: xn9[_R2L[n], :, blk(t, HT)], _nn, cb)
        return steps, lambda p: jnp.concatenate([c[64 * (p // 2):64 * (p // 2) + 64] for c in cb[p % 2]], axis=1)

    def finish_kv(g, src):
        for p in (2 * g, 2 * g + 1):
            keep = (_iota((64, 128), 0) // 32) == (_iota((64, 128), 1) % 2)
            r = _iota((16, 128), 0)
            z = jnp.where((r % 2) == (_iota((16, 128), 1) % 2), src[p, pl.ds(64, 16), :], 0.0)
            zhi = z.astype(BF).astype(F32)
            k = jnp.concatenate([jnp.where(keep, src[p, pl.ds(0, 64), :], 0.0),
                                 jnp.where(r < 2, zhi, jnp.where(r < 4, z - zhi, 0.0))], axis=0)
            kvTb[p] = k.astype(BF)
            kvb[p] = jnp.concatenate([k, jnp.zeros((48, 128), F32)], axis=0).T.astype(BF)

    pair_order = list(range(0, NP, 2)) + list(range(1, NP, 2))
    ones = jnp.ones((16, T), BF)
    zpad = jnp.zeros((48, T), BF)
    out_cp = copy(xv, out_h, osem.at[0])
    dwo_cp = copy(wo, dwo_h, osem.at[1])

    def first(wkT, wqT, dwo_acc, phiq, oT, den, ubuf):
        wo7 = wkT
        kv_acc[...] = jnp.zeros(kv_acc.shape, F32)
        dkv_acc[...] = jnp.zeros(dkv_acc.shape, F32)
        x_cp(0).wait()
        layernorm(0)

        dwo_acc[...] = jnp.zeros(dwo_acc.shape, F32)
        wv_cp.wait()

        def values(i):
            xt = xn[rows(i), :]
            for m in range(4):
                dpT[pl.ds(2 * D + m * T, T), rows(i)] = _nn(xt, wv[:, pl.ds(m * T, T)]).astype(BF).T
                yield

        def p0(i, c):
            x_cp(i + 1).wait()
            _interleave("vvvv", v=values(i))
            layernorm(i + 1)
            return c

        lax.fori_loop(0, NT - 1, p0, 0)
        wk_cp.wait()
        wq_cp.wait()

        def fold_k():
            for g in range(G):
                w = fold(wkT, pl.ds(D + 128 * g, 128), g).astype(BF)
                wf7[1, :, pl.ds(128 * g, 128)] = w[:HD]
                wf7[4, :, pl.ds(128 * g, 128)] = w[HD:]
                yield

        _interleave("ffvffvffvffv", f=fold_k(), v=values(NT - 1))

        def p1(t, c):
            w = fold(wqT, blk(t, 128), t)
            wk = [wf7[n, :, blk(t, 128)].astype(F32) for n in (1, 4)]
            l = _lhs7(lambda i, k: wk[i] if k else w[i * HD:(i + 1) * HD])
            for n in range(7):
                wf7[n, :, blk(t, 128)] = l(n)
            proj, pk = project(wkT, t)

            def k_fwd():
                for p in pair_order:
                    vt = jnp.concatenate([dpT[pl.ds(2 * D + 64 * p, 64), rows(t)], ones], axis=0)
                    phb = _dual_softmax(pk(p))
                    dpT[pl.ds(D + 64 * p, 64), rows(t)] = phb[:64]
                    phik[pl.ds(64 * p, 64), rows(t)] = phb[64:]
                    kv_acc[p] += _nt(vt, phb)
                    yield

            _interleave("pppppphhhhhhp" + "h" * 10, p=proj, h=k_fwd())
            return c

        lax.fori_loop(0, NT, p1, 0)

        for c in late_cp:
            c.wait()

        def prep(g, c):
            finish_kv(g, kv_acc)
            l = _lhs7(lambda a, k: wo[blk(G * a + g, 64), pl.ds(k * HD, HD)])
            for n in range(7):
                wo7[n, blk(g, 64), :] = l(n)
            return c

        lax.fori_loop(0, G, prep, 0, unroll=2)

        def pf(i, c):
            f, t = i // NM, i % NM
            hf = _nn(xn[blk(t, MF), :], w1[:, blk(f, FC)])
            hbuf[blk(t, MF), blk(f, FC)] = hf.astype(BF)
            act = relu(hf)
            cb = _strassen(_lhs7(_blocks(act)),
                           _rhs7(_quad(w2, off(f, FC), 0, HF, HD)), _nn)
            for a, b in _IJ:
                sl = (blk(2 * t + a, HM), pl.ds(b * HD, HD))
                ubuf[sl] = jnp.where(f > 0, ubuf[sl], 0.0) + cb[a][b]
            return c

        lax.fori_loop(0, NF * NM, pf, 0)

        def p2(t, c):
            gate, gds, ds = ([[None, None], [None, None]] for _ in range(3))
            for a, b in _IJ:
                sl = (blk(2 * t + a, HT), pl.ds(b * HD, HD))
                u, go = ubuf[sl], gov[sl].astype(F32)
                sg = jax.nn.sigmoid(u)
                gate[a][b] = u * sg
                ds[a][b] = go * gate[a][b]
                gds[a][b] = go * (sg + gate[a][b] * (1.0 - sg))
            proj, pq = project(wqT, t)

            def q_fwd():
                for p in pair_order:
                    phb = _dual_softmax(pq(p))
                    phiq[p] = phb
                    nd = _nn(kvTb[p], phb)
                    inv = 1.0 / (nd[64:72] + pltpu.roll(nd[64:72], 6, 0) + 1e-6)
                    den[p] = inv
                    oT[pl.ds(64 * p, 64), :] = nd[:64] * _head_rows(inv)
                    yield

            cb = [[None, None], [None, None]]
            _interleave(PLAN_F, p=proj, h=q_fwd(),
                        d=_strassen_steps(lambda n: wo7[n], _rhs7(lambda k, j: ds[j][k]), _nt, cb))
            doT = _join(cb)
            s = _join(_strassen(_lhs7(_blocks(oT[...].T)), lambda n: wo7[_R2L[n]], _nn))

            def q_bwd():
                for p in range(NP):
                    dnum = doT[64 * p:64 * p + 64] * _head_rows(den[p])
                    dden = -_head_sums(dnum * oT[pl.ds(64 * p, 64), :])
                    dnb = jnp.concatenate([dnum, dden], axis=0).astype(BF)
                    phb = phiq[p]
                    dkv_acc[p] += _nt(dnb, phb)
                    dph = _nn(kvb[p], jnp.concatenate([dnb, zpad], axis=0))
                    dpT[pl.ds(64 * p, 64), rows(t)] = _dual_softmax_bwd(phb, dph)
                    yield

            xv[rows(t), :] = (xv[rows(t), :].astype(F32) + s * _join(gate)).astype(BF)
            du = s * _join(gds)
            xn[rows(t), :] = du.astype(BF)
            put_lhs7(du7, t, du.T)

            def dwo_products():
                l, r = _lhs7(_quad(oT, 0, 0, HD, HT)), _rhs7(lambda k, j: ds[k][j])
                for n in range(7):
                    dwo_acc[n] += _nn(l(n), r(n))
                    yield

            _interleave(PLAN_B, h=q_bwd(), d=dwo_products())
            return c

        lax.fori_loop(0, NT, p2, 0)
        out_cp.start()

        def post(g, c):
            finish_kv(g, dkv_acc)
            cb = _strassen(lambda n: n, lambda n: n, lambda n, _: dwo_acc[n, blk(g, 64), :])
            for a, b in _IJ:
                wo[blk(G * a + g, 64), pl.ds(b * HD, HD)] = cb[a][b].astype(BF)
            return c

        lax.fori_loop(0, G, post, 0, unroll=2)
        dwo_cp.start()

    def second(dxnT, dw2s):
        def p3(t, c):
            r = rows(t)
            phi = lambda p: jnp.concatenate([dpT[pl.ds(D + 64 * p, 64), r], phik[pl.ds(64 * p, 64), r]], axis=0)
            dv = [_nn(kvTb[p, pl.ds(0, 64), :], phi(p)).astype(BF) for p in range(NP)]
            acc = []

            def k_bwd():
                for p in range(NP):
                    vs = pl.ds(2 * D + 64 * p, 64)
                    dph = _nn(kvb[p], jnp.concatenate([dpT[vs, r], ones, zpad], axis=0))
                    dpT[pl.ds(D + 64 * p, 64), r] = _dual_softmax_bwd(phi(p), dph)
                    dpT[vs, r] = dv[p]
                    yield

            def v_part():
                for m in range(4):
                    acc.append(_nn(wv[pl.ds(m * (D // 4), D // 4), :], jnp.concatenate(dv, axis=0)))
                    yield

            _interleave("hhhvhhhhvhhhhvhhhhhv", h=k_bwd(), v=v_part())
            dvx = _blocks(jnp.concatenate(acc, axis=0))
            cb = _strassen(lambda n: wf7[n], _rhs7(_quad(dpT, 0, off(t, T), D, HT)), _nn)
            for a, b in _IJ:
                dxnT[pl.ds(a * HD, HD), blk(2 * t + b, HT)] = cb[a][b] + dvx(a, b)
            return c

        lax.fori_loop(0, NT, p3, 0)

        dw2_cp = lambda f: copy(dw2s.at[blk(f, FC)], dw2_h.at[blk(f, FC)], osem.at[8 + f])

        def p5a(f, c):
            cb = _strassen(lambda n: du7[n], tok_rows(hbuf, off(f, FC), HF, relu), _nn)
            for i, j in _IJ:
                dw2s[blk(2 * f + j, HF), pl.ds(i * HD, HD)] = cb[i][j].T.astype(BF)
            dw2_cp(f).start()
            return c

        lax.fori_loop(0, NF, p5a, 0)

        def p5b(i, c):
            f, t = i // NM, i % NM
            da = _strassen(_lhs7(_quad(xn, off(t, MF), 0, HM, HD)),
                           _rhs7(_tr(_quad(w2, off(f, FC), 0, HF, HD))), _nt, True)
            d = [[None, None], [None, None]]
            for a, b in _IJ:
                sl = (blk(2 * t + a, HM), blk(2 * f + b, HF))
                hf = hbuf[sl].astype(F32)
                d[a][b] = jnp.where(hf > 0, da[a][b], jnp.where(hf == 0, 0.5 * da[a][b], 0.0)).astype(BF)
                hbuf[sl] = d[a][b]
            cb = _strassen(_lhs7(_quad(w1, 0, off(f, FC), HD, HF)), _rhs7(lambda k, j: d[j][k]), _nt)
            for a, b in _IJ:
                dxnT[pl.ds(a * HD, HD), blk(2 * t + b, HM)] += cb[a][b]
            return c

        lax.fori_loop(0, NF * NM, p5b, 0)

        def ln_bwd(t):
            r = rows(t)
            dy = dxnT[:, r]
            y = jnp.concatenate([jnp.concatenate([xn9[n, :, blk(t, HT)] for n in ns], axis=1)
                                 for ns in ((0, 7), (8, 4))], axis=0).astype(F32)
            br = dy - jnp.mean(dy, axis=0, keepdims=True) - y * jnp.mean(dy * y, axis=0, keepdims=True)
            rs = jnp.concatenate([rstd[r, :]] * (D // 128), axis=1)
            gov[r, :] = (gov[r, :].astype(F32) + rs * br.T).astype(BF)

        def p4a(i, c):
            for k in range(CB // T):
                ln_bwd(i * (CB // T) + k)
            cb = _strassen(lambda n: xn9[n], tok_cols(dpT, off(i, CB), CB // 2), _nt)
            for a, b in _IJ:
                xn[blk(2 * (i // 2) + a, HD), blk(2 * (i % 2) + b, CB // 2)] = cb[a][b].astype(BF)
            return c

        lax.fori_loop(0, 2 * D // CB, p4a, 0)
        dx_cp = copy(gov, dx_h, osem.at[2])
        dx_cp.start()

        def p4b(i, c):
            def unfold():
                for k in range(CB // 128):
                    g = i * (CB // 128) + k
                    m = None
                    for rs, cs in ((Q, blk(g, 128)), (K, blk(G + g, 128))):
                        gg = xn[rs, blk(g, 128)]
                        xv[rs, blk(g, 128)] = _nn(gg, bd[G + g]).astype(BF)
                        part = lax.dot_general(wqk[:, cs], gg, (((0,), (0,)), ((), ())),
                                               preferred_element_type=F32)
                        m = part if m is None else m + part
                        yield
                    dwphi_ref[blk(g, 128), :] = _nt(jnp.where(hmask, m, 0.0).astype(BF), expand).astype(BF)
                yield

            v = 2 * D // CB + i
            cb = [[None, None], [None, None]]
            _interleave("duuduuduuduududd", u=unfold(), d=_strassen_steps(
                lambda n: xn9[n], tok_cols(dpT, off(v, CB), CB // 2), _nt, cb))
            for a, b in _IJ:
                wv[pl.ds(a * HD, HD), blk(2 * i + b, CB // 2)] = cb[a][b].astype(BF)
            return c

        out_cp.wait()
        lax.fori_loop(0, D // CB, p4b, 0)
        dwqkv_cp = [copy(xv.at[Q], dwqkv_h.at[:, Q], osem.at[3]), copy(xv.at[K], dwqkv_h.at[:, K], osem.at[4]),
                    copy(wv, dwqkv_h.at[:, VV], osem.at[5])]
        for c in dwqkv_cp:
            c.start()

        dw1_cp = lambda f: copy(w1.at[:, blk(f, FC)], dw1_h.at[:, blk(f, FC)], osem.at[8 + NF + f])

        def p5c(f, c):
            cb = _strassen(lambda n: xn9[n], tok_rows(hbuf, off(f, FC), HF), _nn)
            for i, j in _IJ:
                w1[pl.ds(i * HD, HD), blk(2 * f + j, HF)] = cb[i][j].astype(BF)
            dw1_cp(f).start()
            return c

        lax.fori_loop(0, NF, p5c, 0)

        for c in [dwo_cp, dx_cp] + dwqkv_cp:
            c.wait()
        for f in range(NF):
            dw2_cp(f).wait()
            dw1_cp(f).wait()

    V = pltpu.VMEM
    pl.run_scoped(first, V((7, HD, HD), BF), V((7, HD, HD), BF),
                  V((7, HD, HD), F32), V((NP, 128, T), BF),
                  V((D, T), F32), V((NP, 8, T), F32), V((S, D), F32))
    pl.run_scoped(second, V((D, S), F32), V((DFF, D), BF))


@jax.jit
def pallas_recurrent_scan__linear_kernel_hedgehog__dense_activation_relu__prompt_kernel(
    A_x: jax.Array,
    A_wqkv: jax.Array,
    A_w_phi: jax.Array,
    A_wo: jax.Array,
    B_x: jax.Array,
    B_w1: jax.Array,
    B_w2: jax.Array,
    grad_out: jax.Array,
):
    del B_x
    hbm = pl.BlockSpec(memory_space=pl.ANY)
    vmem = pl.BlockSpec(memory_space=pltpu.VMEM)
    sds = jax.ShapeDtypeStruct
    V = pltpu.VMEM
    scratch = [
        V((S, D), BF),
        V((S, D), BF),
        V((D, 2 * D), BF),
        V((D, D), BF),
        V((7, D // 2, D), BF),
        V((D, D), BF),
        V((D, DFF), BF),
        V((DFF, D), BF),
        V((S, D), BF),
        V((9, D // 2, S // 2), BF),
        V((S, 128), F32),
        V((2 * G, 128, 128), BF),
        V((S, DFF), BF),
        V((D, S), BF),
        V((3 * D, S), BF),
        V((7, D // 2, S // 2), BF),
        V((NP, 80, 128), F32),
        V((NP, 80, 128), F32),
        V((NP, 128, 128), BF),
        V((NP, 80, 128), BF),
        pltpu.SemaphoreType.DMA((NT + 7,)),
        pltpu.SemaphoreType.DMA((8 + 2 * NF,)),
    ]
    out, dx, dwqkv, dwphi, dwo, dw1, dw2 = pl.pallas_call(
        _kernel,
        in_specs=[hbm, hbm, vmem, hbm, hbm, hbm, hbm],
        out_specs=[hbm, hbm, hbm, vmem, hbm, hbm, hbm],
        out_shape=[sds((S, D), BF), sds((S, D), BF), sds((D, 3 * D), BF), sds((H * DH, DH), BF),
                   sds((D, D), BF), sds((D, DFF), BF), sds((DFF, D), BF)],
        scratch_shapes=scratch,
        compiler_params=pltpu.CompilerParams(vmem_limit_bytes=126 * 1024 * 1024),
    )(A_x.reshape(S, D), A_wqkv, A_w_phi.reshape(H * DH, DH), A_wo, B_w1, B_w2,
      grad_out.reshape(S, D))
    return (out.reshape(1, S, D), dx.reshape(1, S, D), dwqkv, dwphi.reshape(H, DH, DH),
            dwo, dw1, dw2)
```
